```python
import os as _os
_os.environ.setdefault("JAX_PLATFORMS", "cpu")
import jax
import jax.numpy as jnp

def _softmax(x, axis=-1):
    return jax.nn.softmax(x, axis=axis)
def _gelu(x):
    return jax.nn.gelu(x, approximate=True)
def _silu(x):
    return jax.nn.silu(x)
def _sigmoid(x):
    return jax.nn.sigmoid(x)
def _layernorm(x, axis=-1, eps=1e-5):
    m = jnp.mean(x, axis=axis, keepdims=True)
    v = jnp.var(x, axis=axis, keepdims=True)
    return (x - m) / jnp.sqrt(v + eps)
def _scatter_add(tgt, idx, src, axis=0):
    return tgt.at[idx].add(src)
def _segment_sum(src, seg, n):
    return jax.ops.segment_sum(src, seg, n)
class _Rng:
    def __init__(self, key):
        self._k = key
    def _next(self):
        self._k, sub = jax.random.split(self._k)
        return sub
    def normal(self, shape):
        return jax.random.normal(self._next(), shape, dtype=jnp.bfloat16)
    def randint(self, lo, hi, shape):
        return jax.random.randint(self._next(), shape, lo, hi, dtype=jnp.int32)
    def uniform(self, shape, lo=0.0, hi=1.0):
        return jax.random.uniform(self._next(), shape, jnp.bfloat16, lo, hi)
    def permutation(self, n):
        return jax.random.permutation(self._next(), n)


kernel_name = 'standalone__linear_kernel_hedgehog__prompt'

def setup_inputs():
    _rng = _Rng(jax.random.key(int.from_bytes(__import__("os").urandom(4), "little")))
    _w = (lambda a: (lambda t: t.astype(jnp.bfloat16) if jnp.issubdtype(t.dtype, jnp.floating) else t)(jnp.asarray(a)))
    B, S, D, H = 1, 2048, 1024, 32
    Dh = D // H
    return {
        "x": _w((lambda *s: _rng.normal(s) * 0.4)(B, S, D)),
        "wqkv": _w((lambda *s: _rng.normal(s) * 0.4)(D, 3 * D)),
        "w_phi": _w((lambda *s: _rng.normal(s) * 0.4)(H, Dh, Dh) * (Dh ** -0.5)),
        "wo": _w((lambda *s: _rng.normal(s) * 0.05)(D, D)),
    }

def reference(x, wqkv, w_phi, wo):
    B, S, D = x.shape
    H = 32; Dh = D // H
    qkv = (lambda x, *d: x.transpose(*d))((x @ wqkv).reshape(B, S, 3, H, Dh), 2, 0, 3, 1, 4)
    q, k, v = qkv[0], qkv[1], qkv[2]
    pq = jnp.einsum("bhsd,hdf->bhsf", q, w_phi)
    pk = jnp.einsum("bhsd,hdf->bhsf", k, w_phi)
    phi_q = jnp.concatenate([_softmax(pq, axis=-1), _softmax(-pq, axis=-1)], axis=-1)
    phi_k = jnp.concatenate([_softmax(pk, axis=-1), _softmax(-pk, axis=-1)], axis=-1)
    kv = jnp.einsum("bhsf,bhsd->bhfd", phi_k, v)
    z  = jnp.einsum("bhsf->bhf", phi_k)
    num = jnp.einsum("bhqf,bhfd->bhqd", phi_q, kv)
    den = jnp.einsum("bhqf,bhf->bhq", phi_q, z)[..., None] + 1e-6
    o = num / den
    return (lambda x, *d: x.transpose(*d))(o, 0, 2, 1, 3).reshape(B, S, D) @ wo
```

```python
import functools
import jax
import jax.numpy as jnp
from jax import lax
from jax.experimental import pallas as pl
from jax.experimental.pallas import tpu as pltpu

S, D, H, DH = 2048, 1024, 32, 32
TS = 256
NB = S // TS
F32 = jnp.float32
BF16 = jnp.bfloat16

NT = (((1,), (1,)), ((), ()))
TN = (((0,), (0,)), ((), ()))


def _feature_map(pT):
    p = pT.reshape(H, DH, pT.shape[-1])
    mx = jnp.max(p, axis=1, keepdims=True)
    mn = jnp.min(p, axis=1, keepdims=True)
    ep = jnp.exp(p - mx)
    en = jnp.exp(mn - p)
    pos = ep * (1.0 / jnp.sum(ep, axis=1, keepdims=True))
    neg = en * (1.0 / jnp.sum(en, axis=1, keepdims=True))
    return pos.astype(BF16), neg.astype(BF16)


def _kernel(x_ref, wqkv_ref, wphi_ref, wo_ref, o_ref,
            wqT_ref, wkT_ref, kv_ref, z_ref, l_ref):
    step = pl.program_id(0)

    @pl.when(step == 0)
    def _init():
        r = lax.broadcasted_iota(jnp.int32, (128, 128), 0) // DH
        c = lax.broadcasted_iota(jnp.int32, (128, 128), 1) // DH
        msk = r == c
        for g in range(8):
            wp = wphi_ref[g * 128:(g + 1) * 128, :].astype(F32)
            bd = jnp.concatenate([wp] * 4, axis=1)
            bdT = jnp.where(msk, bd, 0.0).T.astype(BF16)
            wq_g = wqkv_ref[:, g * 128:(g + 1) * 128]
            wk_g = wqkv_ref[:, D + g * 128:D + (g + 1) * 128]
            wqT_ref[g * 128:(g + 1) * 128, :] = lax.dot_general(
                bdT, wq_g, NT, preferred_element_type=F32).astype(BF16)
            wkT_ref[g * 128:(g + 1) * 128, :] = lax.dot_general(
                bdT, wk_g, NT, preferred_element_type=F32).astype(BF16)
        kv_ref[...] = jnp.zeros(kv_ref.shape, F32)
        z_ref[...] = jnp.zeros(z_ref.shape, F32)

    @pl.when(step < NB)
    def _phase0():
        xb = x_ref[...]
        pkT = lax.dot_general(wkT_ref[...], xb, NT, preferred_element_type=F32)
        v = jnp.dot(xb, wqkv_ref[:, 2 * D:3 * D], preferred_element_type=F32).astype(BF16)
        pos, neg = _feature_map(pkT)
        pos = pos.reshape(H * DH, TS)
        neg = neg.reshape(H * DH, TS)
        for g in range(8):
            vg = v[:, g * 128:(g + 1) * 128]
            kv_ref[g, 0] += jnp.dot(pos[g * 128:(g + 1) * 128], vg, preferred_element_type=F32)
            kv_ref[g, 1] += jnp.dot(neg[g * 128:(g + 1) * 128], vg, preferred_element_type=F32)
        zp = pos[:, 0:128].astype(F32)
        zn = neg[:, 0:128].astype(F32)
        for j in range(1, TS // 128):
            zp = zp + pos[:, j * 128:(j + 1) * 128].astype(F32)
            zn = zn + neg[:, j * 128:(j + 1) * 128].astype(F32)
        z_ref[0] += zp
        z_ref[1] += zn

    @pl.when(step == NB)
    def _build():
        zrow_p = jnp.sum(z_ref[0].T, axis=0, keepdims=True)
        zrow_n = jnp.sum(z_ref[1].T, axis=0, keepdims=True)
        r = lax.broadcasted_iota(jnp.int32, (64, 128), 0) // DH
        c = (lax.broadcasted_iota(jnp.int32, (64, 128), 1) % 64) // DH
        msk = r == c
        for g in range(8):
            kvp = kv_ref[g, 0].T
            kvn = kv_ref[g, 1].T
            for hf in range(2):
                lo = hf * 64
                top = jnp.concatenate([kvp[lo:lo + 64, lo:lo + 64], kvn[lo:lo + 64, lo:lo + 64]], axis=1)
                c0 = g * 128 + lo
                zr = jnp.concatenate([zrow_p[:, c0:c0 + 64], zrow_n[:, c0:c0 + 64]], axis=1)
                bot = jnp.broadcast_to(zr, (64, 128))
                l_ref[2 * g + hf, 0:64, :] = jnp.where(msk, top, 0.0).astype(BF16)
                l_ref[2 * g + hf, 64:128, :] = jnp.where(msk, bot, 0.0).astype(BF16)

    @pl.when(step >= NB)
    def _phase1():
        xb = x_ref[...]
        pqT = lax.dot_general(wqT_ref[...], xb, NT, preferred_element_type=F32)
        pos, neg = _feature_map(pqT)
        outs = []
        for gg in range(16):
            rhs = jnp.concatenate([pos[2 * gg:2 * gg + 2].reshape(64, TS),
                                   neg[2 * gg:2 * gg + 2].reshape(64, TS)], axis=0)
            a = jnp.dot(l_ref[gg], rhs, preferred_element_type=F32)
            oT = a[:64] / (a[64:] + 1e-6)
            outs.append(oT.astype(BF16))
        oT = jnp.concatenate(outs, axis=0)
        o_ref[...] = lax.dot_general(oT, wo_ref[...], TN, preferred_element_type=F32).astype(BF16)


@jax.jit
def pallas_standalone__linear_kernel_hedgehog__prompt_kernel(x, wqkv, w_phi, wo):
    x2 = x.reshape(S, D)
    wphi2 = w_phi.reshape(H * DH, DH)
    out = pl.pallas_call(
        _kernel,
        grid=(2 * NB,),
        in_specs=[
            pl.BlockSpec((TS, D), lambda i: (i % NB, 0)),
            pl.BlockSpec((D, 3 * D), lambda i: (0, 0)),
            pl.BlockSpec((H * DH, DH), lambda i: (0, 0)),
            pl.BlockSpec((D, D), lambda i: (0, 0)),
        ],
        out_specs=pl.BlockSpec((TS, D), lambda i: (jnp.maximum(i - NB, 0), 0)),
        out_shape=jax.ShapeDtypeStruct((S, D), BF16),
        scratch_shapes=[
            pltpu.VMEM((D, D), BF16),
            pltpu.VMEM((D, D), BF16),
            pltpu.VMEM((8, 2, 128, 128), F32),
            pltpu.VMEM((2, H * DH, 128), F32),
            pltpu.VMEM((16, 128, 128), BF16),
        ],
        compiler_params=pltpu.CompilerParams(
            dimension_semantics=("arbitrary",),
            vmem_limit_bytes=100 * 1024 * 1024,
        ),
    )(x2, wqkv, wphi2, wo)
    return out.reshape(1, S, D)
```

```python
import jax
import jax.numpy as jnp
from jax import lax
from jax.experimental import pallas as pl
from jax.experimental.pallas import tpu as pltpu

S, D, H, DH = 2048, 1024, 32, 32
TS = 256
NB = S // TS
NC = 4
CH = D // NC
SWP = 1
F32 = jnp.float32
BF16 = jnp.bfloat16

NT = (((1,), (1,)), ((), ()))
TN = (((0,), (0,)), ((), ()))


def _feature_map(pT):
    p = pT.reshape(H, DH, pT.shape[-1])
    mx = jnp.max(p, axis=1, keepdims=True)
    mn = jnp.min(p, axis=1, keepdims=True)
    ep = jnp.exp(p - mx)
    en = jnp.exp(mn - p)
    pos = ep * (1.0 / jnp.sum(ep, axis=1, keepdims=True))
    neg = en * (1.0 / jnp.sum(en, axis=1, keepdims=True))
    return pos, neg


def _group_rhs(pos, neg, gg):
    n = pos.shape[-1]
    return jnp.concatenate([pos[2 * gg:2 * gg + 2].reshape(64, n),
                            neg[2 * gg:2 * gg + 2].reshape(64, n)], axis=0)


def _lane_fold(a):
    out = a[:, 0:128]
    for j in range(1, a.shape[-1] // 128):
        out = out + a[:, j * 128:(j + 1) * 128]
    return out


def _kernel(x_hbm, wqkv_hbm, wphi_hbm, wo_hbm, o_hbm,
            x_v, w_v, wphi_v, wo_v, out_v, bd_v, wa_v, wq_v, y0_v, lacc_v, l_v, z_v, ot_v,
            sem_x, sem_w, sem_misc, sem_o):

    def x_copy(i):
        return pltpu.make_async_copy(x_hbm.at[pl.ds(i * TS, TS), :], x_v.at[pl.ds(i * TS, TS), :], sem_x.at[i])

    def w_copy(c):
        return pltpu.make_async_copy(wqkv_hbm.at[pl.ds(c * CH, CH), pl.ds(D, 2 * D)],
                                     w_v.at[pl.ds(c * CH, CH), pl.ds(D, 2 * D)], sem_w.at[c])

    wphi_copy = pltpu.make_async_copy(wphi_hbm, wphi_v, sem_misc.at[0])
    wq_copy = pltpu.make_async_copy(wqkv_hbm.at[:, pl.ds(0, D)], w_v.at[:, pl.ds(0, D)], sem_misc.at[1])
    wo_copy = pltpu.make_async_copy(wo_hbm, wo_v, sem_misc.at[2])

    def o_copy(i):
        return pltpu.make_async_copy(out_v.at[pl.ds(i * TS, TS), :], o_hbm.at[pl.ds(i * TS, TS), :], sem_o.at[i])

    def issue_w(c, carry):
        @pl.when(c == 0)
        def _():
            wphi_copy.start()
        w_copy(c).start()
        @pl.when(c == 0)
        def _():
            x_copy(0).start()
        return carry

    lax.fori_loop(0, NC, issue_w, 0)

    def issue_rest(i, carry):
        x_copy(i).start()
        @pl.when(i == NB - 1)
        def _():
            wq_copy.start()
        return carry

    wphi_copy.wait()
    r = lax.broadcasted_iota(jnp.int32, (128, 128), 0) // DH
    c_ = lax.broadcasted_iota(jnp.int32, (128, 128), 1) // DH
    msk = r == c_
    for g in range(8):
        wp = wphi_v[g * 128:(g + 1) * 128, :].astype(F32)
        bd = jnp.concatenate([wp] * 4, axis=1)
        bd_v[g] = jnp.where(msk, bd, 0.0).T.astype(BF16)

    lacc_v[...] = jnp.zeros(lacc_v.shape, F32)
    z_v[...] = jnp.zeros(z_v.shape, F32)

    def kv_update(y):
        pos, neg = _feature_map(y[:D])
        z_v[0] += _lane_fold(pos.reshape(D, TS))
        z_v[1] += _lane_fold(neg.reshape(D, TS))
        pos = pos.astype(BF16)
        neg = neg.astype(BF16)
        vT = y[D:].astype(BF16)
        for gg in range(16):
            lacc_v[gg] += lax.dot_general(vT[gg * 64:(gg + 1) * 64], _group_rhs(pos, neg, gg), NT,
                                          preferred_element_type=F32)

    for c in range(NC):
        w_copy(c).wait()
        if c == NC - 1:
            lax.fori_loop(1, NB, issue_rest, 0)
            wo_copy.start()
        cs = slice(c * CH, (c + 1) * CH)
        parts = []
        for g in range(8):
            wk = w_v[cs, D + g * 128:D + (g + 1) * 128]
            parts.append(lax.dot_general(bd_v[g], wk, NT, preferred_element_type=F32).astype(BF16))
        for g in range(8):
            parts.append(w_v[cs, 2 * D + g * 128:2 * D + (g + 1) * 128].T)
        cur = jnp.concatenate(parts, axis=0)
        wa_v[:, cs] = cur
        if c == 0:
            x_copy(0).wait()
        part = lax.dot_general(cur, x_v[0:TS, cs], NT, preferred_element_type=F32)
        if c == 0:
            y0_v[...] = part
        elif c < NC - 1:
            y0_v[...] += part
        else:
            kv_update(y0_v[...] + part)

    def p0_body(i, carry):
        x_copy(i).wait()
        xb = x_v[pl.ds(pl.multiple_of(i * TS, TS), TS), :]
        kv_update(lax.dot_general(wa_v[...], xb, NT, preferred_element_type=F32))
        return carry

    lax.fori_loop(1, NB, p0_body, 0)

    rr = lax.broadcasted_iota(jnp.int32, (64, 128), 0) // DH
    cc = (lax.broadcasted_iota(jnp.int32, (64, 128), 1) % 64) // DH
    lmsk = rr == cc
    for gg in range(16):
        l_v[gg] = jnp.where(lmsk, lacc_v[gg], 0.0).astype(BF16)
    for s_ in range(2):
        z_v[s_] = jnp.broadcast_to(jnp.sum(z_v[s_], axis=1, keepdims=True), (D, 128))

    wq_copy.wait()
    for g in range(8):
        wq_v[g * 128:(g + 1) * 128, :] = lax.dot_general(
            bd_v[g], w_v[:, g * 128:(g + 1) * 128], NT, preferred_element_type=F32).astype(BF16)
    wo_copy.wait()

    def q_mm(i):
        row = pl.multiple_of(i * TS, TS)
        xb = x_v[pl.ds(row, TS), :]
        return lax.dot_general(wq_v[...], xb, NT, preferred_element_type=F32)

    def q_rest(y):
        pos, neg = _feature_map(y)
        zp = jnp.concatenate([z_v[0]] * (TS // 128), axis=1).reshape(H, DH, TS)
        zn = jnp.concatenate([z_v[1]] * (TS // 128), axis=1).reshape(H, DH, TS)
        den = jnp.sum(pos * zp + neg * zn, axis=1, keepdims=True) + 1e-6
        rden = 1.0 / den
        pos = pos.astype(BF16)
        neg = neg.astype(BF16)
        outs = []
        for gg in range(16):
            a = jnp.dot(l_v[gg], _group_rhs(pos, neg, gg), preferred_element_type=F32)
            outs.append((a[0:32] * rden[2 * gg]).astype(BF16))
            outs.append((a[32:64] * rden[2 * gg + 1]).astype(BF16))
        return jnp.concatenate(outs, axis=0)

    def o_part(i, oT):
        row = pl.multiple_of(i * TS, TS)
        out_v[pl.ds(row, TS), :] = lax.dot_general(
            oT, wo_v[...], TN, preferred_element_type=F32).astype(BF16)

    if SWP:
        ot_v[0] = q_rest(q_mm(0))

        def p1_body(i, carry):
            prev_ot = ot_v[(i - 1) % 2]
            y = q_mm(i)
            o_part(i - 1, prev_ot)
            ot_v[i % 2] = q_rest(y)
            o_copy(i - 1).start()
            return carry

        lax.fori_loop(1, NB, p1_body, 0)
        o_part(NB - 1, ot_v[(NB - 1) % 2])
        o_copy(NB - 1).start()
    else:
        def p1_body(i, carry):
            o_part(i, q_rest(q_mm(i)))
            o_copy(i).start()
            return carry

        lax.fori_loop(0, NB, p1_body, 0)
    for i in range(NB):
        o_copy(i).wait()


@jax.jit
def pallas_standalone__linear_kernel_hedgehog__prompt_kernel(x, wqkv, w_phi, wo):
    x2 = x.reshape(S, D)
    wphi2 = w_phi.reshape(H * DH, DH)
    out = pl.pallas_call(
        _kernel,
        in_specs=[pl.BlockSpec(memory_space=pl.ANY)] * 4,
        out_specs=pl.BlockSpec(memory_space=pl.ANY),
        out_shape=jax.ShapeDtypeStruct((S, D), BF16),
        scratch_shapes=[
            pltpu.VMEM((S, D), BF16),
            pltpu.VMEM((D, 3 * D), BF16),
            pltpu.VMEM((H * DH, DH), BF16),
            pltpu.VMEM((D, D), BF16),
            pltpu.VMEM((S, D), BF16),
            pltpu.VMEM((8, 128, 128), BF16),
            pltpu.VMEM((2 * D, D), BF16),
            pltpu.VMEM((D, D), BF16),
            pltpu.VMEM((2 * D, TS), F32),
            pltpu.VMEM((16, 64, 128), F32),
            pltpu.VMEM((16, 64, 128), BF16),
            pltpu.VMEM((2, D, 128), F32),
            pltpu.VMEM((2, D, TS), BF16),
            pltpu.SemaphoreType.DMA((NB,)),
            pltpu.SemaphoreType.DMA((NC,)),
            pltpu.SemaphoreType.DMA((3,)),
            pltpu.SemaphoreType.DMA((NB,)),
        ],
        compiler_params=pltpu.CompilerParams(
            vmem_limit_bytes=100 * 1024 * 1024,
        ),
    )(x2, wqkv, wphi2, wo)
    return out.reshape(1, S, D)
```

```python
import jax
import jax.numpy as jnp
from jax import lax
from jax.experimental import pallas as pl
from jax.experimental.pallas import tpu as pltpu

S, D, H, DH = 2048, 1024, 32, 32
TS = 256
NB = S // TS
CHUNKS = (128, 128, 256, 256, 256)
NC = len(CHUNKS)
COFF = [sum(CHUNKS[:i]) for i in range(NC)]
NSPLIT = 4
XPOS = 1
F32 = jnp.float32
BF16 = jnp.bfloat16

NT = (((1,), (1,)), ((), ()))
TN = (((0,), (0,)), ((), ()))


def _feature_map(pT):
    p = pT.reshape(H, DH, pT.shape[-1])
    mx = jnp.max(p, axis=1, keepdims=True)
    mn = jnp.min(p, axis=1, keepdims=True)
    ep = jnp.exp(p - mx)
    en = jnp.exp(mn - p)
    pos = ep * (1.0 / jnp.sum(ep, axis=1, keepdims=True))
    neg = en * (1.0 / jnp.sum(en, axis=1, keepdims=True))
    return pos, neg


def _group_rhs(pos, neg, gg):
    n = pos.shape[-1]
    return jnp.concatenate([pos[2 * gg:2 * gg + 2].reshape(64, n),
                            neg[2 * gg:2 * gg + 2].reshape(64, n)], axis=0)


def _lane_fold(a):
    out = a[:, 0:128]
    for j in range(1, a.shape[-1] // 128):
        out = out + a[:, j * 128:(j + 1) * 128]
    return out


def _ordered_start(copies):
    def body(k, carry):
        for idx, cp in enumerate(copies):
            @pl.when(k == idx)
            def _():
                cp.start()
        return carry
    lax.fori_loop(0, len(copies), body, 0)


def _kernel(x_hbm, wqkv_hbm, wphi_hbm, wo_hbm, o_hbm,
            x_v, w_v, wphi_v, wo_v, out_v, bd_v, wa_v, wq_v, y0_v, lacc_v, l_v, z_v, ot_v,
            sem_x, sem_w, sem_misc, sem_o):

    def x_copy(i):
        return pltpu.make_async_copy(x_hbm.at[pl.ds(i * TS, TS), :], x_v.at[pl.ds(i * TS, TS), :], sem_x.at[i])

    def w_copy(c):
        return pltpu.make_async_copy(wqkv_hbm.at[pl.ds(COFF[c], CHUNKS[c]), pl.ds(D, 2 * D)],
                                     w_v.at[pl.ds(COFF[c], CHUNKS[c]), pl.ds(D, 2 * D)], sem_w.at[c])

    wphi_copy = pltpu.make_async_copy(wphi_hbm, wphi_v, sem_misc.at[0])
    wq_copy = pltpu.make_async_copy(wqkv_hbm.at[:, pl.ds(0, D)], w_v.at[:, pl.ds(0, D)], sem_misc.at[1])
    wo_copy = pltpu.make_async_copy(wo_hbm, wo_v, sem_misc.at[2])

    def o_copy(i):
        return pltpu.make_async_copy(out_v.at[pl.ds(i * TS, TS), :], o_hbm.at[pl.ds(i * TS, TS), :], sem_o.at[i])

    def last_copy(j):
        cw = D // NSPLIT
        r0 = (NB - 1) * TS
        return pltpu.make_async_copy(out_v.at[pl.ds(r0, TS), pl.ds(j * cw, cw)],
                                     o_hbm.at[pl.ds(r0, TS), pl.ds(j * cw, cw)], sem_o.at[NB - 1 + j])

    first = [wphi_copy] + [w_copy(c) for c in range(XPOS)] + [x_copy(0)] + [w_copy(c) for c in range(XPOS, NC)]
    _ordered_start(first)

    wphi_copy.wait()
    hcol = lax.broadcasted_iota(jnp.int32, (DH, 128), 1) // DH
    for g in range(8):
        wT = wphi_v[g * 128:(g + 1) * 128, :].astype(F32).T
        bd_v[g] = jnp.concatenate([jnp.where(hcol == hh, wT, 0.0) for hh in range(4)], axis=0).astype(BF16)

    lacc_v[...] = jnp.zeros(lacc_v.shape, F32)
    z_v[...] = jnp.zeros(z_v.shape, F32)

    def kv_update(y):
        pos, neg = _feature_map(y[:D])
        z_v[0] += _lane_fold(pos.reshape(D, TS))
        z_v[1] += _lane_fold(neg.reshape(D, TS))
        pos = pos.astype(BF16)
        neg = neg.astype(BF16)
        vT = y[D:].astype(BF16)
        for gg in range(16):
            lacc_v[gg] += lax.dot_general(vT[gg * 64:(gg + 1) * 64], _group_rhs(pos, neg, gg), NT,
                                          preferred_element_type=F32)

    for c in range(NC):
        w_copy(c).wait()
        if c == NC - 1:
            _ordered_start([x_copy(i) for i in range(1, NB)] + [wq_copy, wo_copy])
        cs = slice(COFF[c], COFF[c] + CHUNKS[c])
        kparts = []
        for g in range(8):
            wk = w_v[cs, D + g * 128:D + (g + 1) * 128]
            kparts.append(lax.dot_general(bd_v[g], wk, NT, preferred_element_type=F32).astype(BF16))
        vparts = [w_v[cs, 2 * D + g * 128:2 * D + (g + 1) * 128].T for g in range(8)]
        kcur = jnp.concatenate(kparts, axis=0)
        vcur = jnp.concatenate(vparts, axis=0)
        wa_v[0:D, cs] = kcur
        wa_v[D:2 * D, cs] = vcur
        if c == 0:
            x_copy(0).wait()
        xc = x_v[0:TS, cs]
        part = jnp.concatenate([lax.dot_general(kcur, xc, NT, preferred_element_type=F32),
                                lax.dot_general(vcur, xc, NT, preferred_element_type=F32)], axis=0)
        if c == 0:
            y0_v[...] = part
        elif c < NC - 1:
            y0_v[...] += part
        else:
            kv_update(y0_v[...] + part)

    def p0_body(i, carry):
        x_copy(i).wait()
        xb = x_v[pl.ds(pl.multiple_of(i * TS, TS), TS), :]
        kv_update(lax.dot_general(wa_v[...], xb, NT, preferred_element_type=F32))
        return carry

    lax.fori_loop(1, NB, p0_body, 0)

    wq_copy.wait()
    wo_copy.wait()
    for g in range(8):
        wq_v[g * 128:(g + 1) * 128, :] = lax.dot_general(
            bd_v[g], w_v[:, g * 128:(g + 1) * 128], NT, preferred_element_type=F32).astype(BF16)

    rr = lax.broadcasted_iota(jnp.int32, (64, 128), 0) // DH
    cc = (lax.broadcasted_iota(jnp.int32, (64, 128), 1) % 64) // DH
    lmsk = rr == cc
    for gg in range(16):
        l_v[gg] = jnp.where(lmsk, lacc_v[gg], 0.0).astype(BF16)
    for s_ in range(2):
        z_v[s_] = jnp.broadcast_to(jnp.sum(z_v[s_], axis=1, keepdims=True), (D, 128))

    def q_mm(i):
        row = pl.multiple_of(i * TS, TS)
        xb = x_v[pl.ds(row, TS), :]
        return lax.dot_general(wq_v[...], xb, NT, preferred_element_type=F32)

    def q_rest(y):
        pos, neg = _feature_map(y)
        zp = jnp.concatenate([z_v[0]] * (TS // 128), axis=1).reshape(H, DH, TS)
        zn = jnp.concatenate([z_v[1]] * (TS // 128), axis=1).reshape(H, DH, TS)
        den = jnp.sum(pos * zp + neg * zn, axis=1, keepdims=True) + 1e-6
        rden = 1.0 / den
        pos = pos.astype(BF16)
        neg = neg.astype(BF16)
        outs = []
        for gg in range(16):
            a = jnp.dot(l_v[gg], _group_rhs(pos, neg, gg), preferred_element_type=F32)
            outs.append((a[0:32] * rden[2 * gg]).astype(BF16))
            outs.append((a[32:64] * rden[2 * gg + 1]).astype(BF16))
        return jnp.concatenate(outs, axis=0)

    def o_part(i, oT):
        row = pl.multiple_of(i * TS, TS)
        out_v[pl.ds(row, TS), :] = lax.dot_general(
            oT, wo_v[...], TN, preferred_element_type=F32).astype(BF16)

    ot_v[0] = q_rest(q_mm(0))

    def p1_body(i, carry):
        prev_ot = ot_v[(i - 1) % 2]
        y = q_mm(i)
        o_part(i - 1, prev_ot)
        ot_v[i % 2] = q_rest(y)
        o_copy(i - 1).start()
        return carry

    lax.fori_loop(1, NB, p1_body, 0)

    oT = ot_v[(NB - 1) % 2]
    r0 = (NB - 1) * TS
    for j in range(NSPLIT):
        cw = D // NSPLIT
        out_v[r0:r0 + TS, j * cw:(j + 1) * cw] = lax.dot_general(
            oT, wo_v[:, j * cw:(j + 1) * cw], TN, preferred_element_type=F32).astype(BF16)
        last_copy(j).start()
    for i in range(NB - 1):
        o_copy(i).wait()
    for j in range(NSPLIT):
        last_copy(j).wait()


@jax.jit
def pallas_standalone__linear_kernel_hedgehog__prompt_kernel(x, wqkv, w_phi, wo):
    x2 = x.reshape(S, D)
    wphi2 = w_phi.reshape(H * DH, DH)
    out = pl.pallas_call(
        _kernel,
        in_specs=[pl.BlockSpec(memory_space=pl.ANY)] * 4,
        out_specs=pl.BlockSpec(memory_space=pl.ANY),
        out_shape=jax.ShapeDtypeStruct((S, D), BF16),
        scratch_shapes=[
            pltpu.VMEM((S, D), BF16),
            pltpu.VMEM((D, 3 * D), BF16),
            pltpu.VMEM((H * DH, DH), BF16),
            pltpu.VMEM((D, D), BF16),
            pltpu.VMEM((S, D), BF16),
            pltpu.VMEM((8, 128, 128), BF16),
            pltpu.VMEM((2 * D, D), BF16),
            pltpu.VMEM((D, D), BF16),
            pltpu.VMEM((2 * D, TS), F32),
            pltpu.VMEM((16, 64, 128), F32),
            pltpu.VMEM((16, 64, 128), BF16),
            pltpu.VMEM((2, D, 128), F32),
            pltpu.VMEM((2, D, TS), BF16),
            pltpu.SemaphoreType.DMA((NB,)),
            pltpu.SemaphoreType.DMA((NC,)),
            pltpu.SemaphoreType.DMA((3,)),
            pltpu.SemaphoreType.DMA((NB - 1 + NSPLIT,)),
        ],
        compiler_params=pltpu.CompilerParams(
            vmem_limit_bytes=100 * 1024 * 1024,
        ),
    )(x2, wqkv, wphi2, wo)
    return out.reshape(1, S, D)
```
